```python
import os as _os
_os.environ.setdefault("JAX_PLATFORMS", "cpu")
import jax
import jax.numpy as jnp

def _softmax(x, axis=-1):
    return jax.nn.softmax(x, axis=axis)
def _gelu(x):
    return jax.nn.gelu(x, approximate=True)
def _silu(x):
    return jax.nn.silu(x)
def _sigmoid(x):
    return jax.nn.sigmoid(x)
def _layernorm(x, axis=-1, eps=1e-5):
    m = jnp.mean(x, axis=axis, keepdims=True)
    v = jnp.var(x, axis=axis, keepdims=True)
    return (x - m) / jnp.sqrt(v + eps)
def _scatter_add(tgt, idx, src, axis=0):
    return tgt.at[idx].add(src)
def _segment_sum(src, seg, n):
    return jax.ops.segment_sum(src, seg, n)
class _Rng:
    def __init__(self, key):
        self._k = key
    def _next(self):
        self._k, sub = jax.random.split(self._k)
        return sub
    def normal(self, shape):
        return jax.random.normal(self._next(), shape, dtype=jnp.bfloat16)
    def randint(self, lo, hi, shape):
        return jax.random.randint(self._next(), shape, lo, hi, dtype=jnp.int32)
    def uniform(self, shape, lo=0.0, hi=1.0):
        return jax.random.uniform(self._next(), shape, jnp.bfloat16, lo, hi)
    def permutation(self, n):
        return jax.random.permutation(self._next(), n)


kernel_name = 'gated_mix__sliding_local_dilated__moe_arch_mod__prompt'

def setup_inputs():
    _rng = _Rng(jax.random.key(int.from_bytes(__import__("os").urandom(4), "little")))
    _w = (lambda a: (lambda t: t.astype(jnp.bfloat16) if jnp.issubdtype(t.dtype, jnp.floating) else t)(jnp.asarray(a)))
    def _A_setup():
        B, S, D = 1, 2048, 640
        return {
            "x": _w((lambda *s: _rng.normal(s) * 0.05)(B, S, D)),
            "wqkv": _w((lambda *s: _rng.normal(s) * 0.8)(D, 3 * D)),
            "wo": _w((lambda *s: _rng.normal(s) * 0.05)(D, D)),
        }
    _A_in = _A_setup()

    def _B_setup():
        B, S, D, F, C = 1, 2048, 640, 1728, 1
        return {
            "x": _w((lambda *s: _rng.normal(s) * 0.05)(B, S, D)),
            "w_r": _w((lambda *s: _rng.normal(s) * 1.6)(D)),
            "w_gate": _w((lambda *s: _rng.normal(s) * 0.4)(D, F)),
            "w_up": _w((lambda *s: _rng.normal(s) * 0.4)(D, F)),
            "w_down": _w((lambda *s: _rng.normal(s) * 0.4)(F, D)),
        }
    _B_in = _B_setup()

    return {
        "A_x": _A_in["x"],
        "A_wqkv": _A_in["wqkv"],
        "A_wo": _A_in["wo"],
        "B_x": _B_in["x"],
        "B_w_r": _B_in["w_r"],
        "B_w_gate": _B_in["w_gate"],
        "B_w_up": _B_in["w_up"],
        "B_w_down": _B_in["w_down"],
        "gate_w": _w((lambda *s: _rng.normal(s) * 0.05)(640) * 16.0),
    }

def reference(A_x, A_wqkv, A_wo, B_x, B_w_r, B_w_gate, B_w_up, B_w_down, gate_w):
    def _A_ref(x, wqkv, wo):
        B, S, D = x.shape
        H = 32; Dh = D // H
        W, dil = 8, 2
        qkv = (lambda x, *d: x.transpose(*d))((x @ wqkv).reshape(B, S, 3, H, Dh), 2, 0, 3, 1, 4)
        q, k, v = qkv[0], qkv[1], qkv[2]
        scale = Dh ** -0.5
        pos = jnp.arange(S)
        off = jnp.arange(W) * dil
        idx = pos[:, None] - off[None, :]
        mask = idx >= 0
        idx_c = jnp.where(mask, idx, 0).reshape(-1)
        kg = k[:, :, idx_c, :].reshape(B, H, S, W, Dh)
        vg = v[:, :, idx_c, :].reshape(B, H, S, W, Dh)
        logits = jnp.einsum("bhsd,bhswd->bhsw", q, kg) * scale
        logits = jnp.where(mask[None, None, :, :], logits, -1e9)
        attn = _softmax(logits, axis=-1)
        o = jnp.einsum("bhsw,bhswd->bhsd", attn, vg)
        return (lambda x, *d: x.transpose(*d))(o, 0, 2, 1, 3).reshape(B, S, D) @ wo

    def _B_ref(x, w_r, w_gate, w_up, w_down):
        B, S, D = x.shape
        C = 1
        r = x @ w_r
        idx = jnp.argsort(-r, axis=-1)[:, :C]
        idx_e = jnp.repeat(idx.reshape(B, C, 1), D, axis=2)
        x_sel = jnp.take_along_axis(x, idx_e, axis=1)
        g = _silu(x_sel @ w_gate)
        u = x_sel @ w_up
        y = (g * u) @ w_down
        r_sel = _sigmoid(jnp.take_along_axis(r, idx, axis=1))
        y = y * r_sel.reshape(B, C, 1)
        b_off = (jnp.arange(B) * S).reshape(B, 1)
        flat_idx = (idx + b_off).reshape(B * C)
        zero = (x * 0.0).reshape(B * S, D)
        upd = _scatter_add(zero, flat_idx, y.reshape(B * C, D), axis=0)
        return x + upd.reshape(B, S, D)

    x = A_x
    g = _sigmoid((x * gate_w).sum(-1, keepdims=True))
    a = _A_ref(x, A_wqkv, A_wo)
    b = _B_ref(x, B_w_r, B_w_gate, B_w_up, B_w_down)
    return g * a + (1 - g) * b
```

```python
import functools
import math
import numpy as np
import jax
import jax.numpy as jnp
from jax import lax
import jax.experimental.pallas as pl
import jax.experimental.pallas.tpu as pltpu

S, D, H, DH, W, DIL, F = 2048, 640, 32, 20, 8, 2, 1728
NT = D // 128
HALO = 16
F32, BF16, U32 = jnp.float32, jnp.bfloat16, jnp.uint32
NT_DIMS = (((1,), (1,)), ((), ()))
ORDER = (1, 2, 0)


def sigmoid(t):
    return 0.5 * jnp.tanh(0.5 * t) + 0.5


def split(seq, n):
    seq = list(seq)
    return [seq[len(seq) * i // n:len(seq) * (i + 1) // n] for i in range(n)]


def make_kernel(CM, RC, FC, NP, P0, x_at, f_at, r_rng, gu_rng, dn_rng, ocuts, tie, prio, scopes, LA, LM, OL, CU, TF, LE):
    NC = S // CM
    X0 = P0 * CM
    ocuts = (0,) + tuple(ocuts) + (S,)
    NO = len(ocuts) - 1

    def scope(name):
        import contextlib
        return jax.named_scope(name) if scopes else contextlib.nullcontext()

    def kernel(x_hbm, wqkv_hbm, wo_hbm, wr_ref, wg_hbm, wu_hbm, wd_hbm, gw_ref, out_hbm,
               x_v, wqkv_v, wo_v, wg_v, wu_v, wd_v, t_s, wt_s, wop_s, out_v,
               sem_w, sem_x, sem_f, sem_o, sem_p, *kv):
        k_s, v_s = kv[:NC], kv[NC:]
        cp_w = [pltpu.make_async_copy(wqkv_hbm.at[:, p * D:(p + 1) * D], wqkv_v.at[p], sem_w.at[p]) for p in range(3)]
        cp_wo = pltpu.make_async_copy(wo_hbm, wo_v, sem_w.at[3])
        cp_x0 = pltpu.make_async_copy(x_hbm.at[pl.ds(0, X0)], x_v.at[pl.ds(0, X0)], sem_x.at[0])
        X1 = f_at * CM
        cp_x1 = pltpu.make_async_copy(x_hbm.at[pl.ds(X0, X1 - X0)], x_v.at[pl.ds(X0, X1 - X0)], sem_x.at[1])
        cp_x2 = pltpu.make_async_copy(x_hbm.at[pl.ds(X1, S - X1)], x_v.at[pl.ds(X1, S - X1)], sem_x.at[2])
        cp_f = [pltpu.make_async_copy(a, b, sem_f.at[i]) for i, (a, b) in enumerate(((wg_hbm, wg_v), (wu_hbm, wu_v), (wd_hbm, wd_v)))]
        cp_o = [pltpu.make_async_copy(out_v.at[pl.ds(a, b - a)], out_hbm.at[pl.ds(a, b - a)], sem_o.at[i])
                for i, (a, b) in enumerate(zip(ocuts[:-1], ocuts[1:]))]

        cp_w[ORDER[0]].start()
        cp_x0.start()
        cp_w[ORDER[1]].start(priority=prio)

        def permute_rows(slot, dst, base):
            for j in range(NT):
                for d in range(DH):
                    dst[pl.ds((base + d * H) // 2, H // 2), j * 128:(j + 1) * 128] = pltpu.bitcast(
                        t_s[slot, j, pl.ds(d, H, stride=DH), :].astype(BF16), U32)

        for j in range(NT):
            k_s[0][j, 0:HALO, :] = jnp.zeros((HALO, 128), F32)
            v_s[0][j, 0:HALO, :] = jnp.zeros((HALO, 128), F32)
        wr = wr_ref[...].astype(F32).reshape(1, D)
        gw = gw_ref[...].astype(F32).reshape(1, D)
        c = (DH ** -0.5) * math.log2(math.e)

        def wait_w(n):
            with scope('wait_w%d' % n):
                cp_w[ORDER[n]].wait()
            if n == 0:
                cp_w[ORDER[2]].start(priority=prio)
            if n == x_at:
                cp_wo.start(priority=prio)
                cp_x1.start(priority=prio)

        def prep_w(n):
            p = ORDER[n]
            for j in range(NT):
                t_s[n, j] = wqkv_v[p, j * 128:(j + 1) * 128, :].astype(F32).T
            permute_rows(n, wt_s, p * D)

        def prep_wo():
            for j in range(NT):
                t_s[0, j] = wo_v[:, j * 128:(j + 1) * 128].astype(F32)
            permute_rows(0, wop_s, 0)

        st = dict(m=jnp.full((8, 1), -jnp.inf, F32), bi=jnp.zeros((8, 1), jnp.int32), hs={}, acc=jnp.zeros((8, D), F32))
        sub = lax.broadcasted_iota(jnp.int32, (8, 1), 0)

        def router_tile(t):
            xs = x_v[t * 16:(t + 1) * 16, :].astype(F32)
            r = jnp.sum(xs * wr, axis=-1, keepdims=True).astype(BF16).astype(F32)
            for hh in range(2):
                rr = r[hh * 8:(hh + 1) * 8]
                better = rr > st['m']
                st['m'] = jnp.where(better, rr, st['m'])
                st['bi'] = jnp.where(better, sub + (t * 16 + hh * 8), st['bi'])
            return [pltpu.bitcast(jnp.broadcast_to(st['bi'], (8, 128)), U32)]

        def router_fin():
            m, bi = st['m'], st['bi']
            mm = jnp.max(m, axis=0, keepdims=True)
            ii = jnp.min(jnp.where(m == mm, bi, S), axis=0, keepdims=True)
            idx = jnp.clip(ii[0, 0], 0, S - 1)
            t0 = pl.multiple_of((idx // 16) * 16, 16)
            xt = x_v[pl.ds(t0, 16), :].astype(F32)
            sel = (t0 + lax.broadcasted_iota(jnp.int32, (16, 1), 0)) == idx
            st.update(mm=mm, idx=idx, t0=t0, sel=sel, xt=xt,
                      xrow=jnp.sum(jnp.where(sel, xt, 0.0), axis=0, keepdims=True))
            return []

        def gate_up(f0):
            gg = jnp.sum(wg_v[f0:f0 + FC, :].astype(F32) * st['xrow'], axis=-1, keepdims=True)
            uu = jnp.sum(wu_v[f0:f0 + FC, :].astype(F32) * st['xrow'], axis=-1, keepdims=True)
            hh = gg * sigmoid(gg) * uu
            t = wd_v[f0:f0 + FC, :].astype(F32) * hh
            for u in range(FC // 8):
                st['acc'] = st['acc'] + t[u * 8:(u + 1) * 8]
            return [pltpu.bitcast(st['acc'][:, j * 128:(j + 1) * 128], U32) for j in range(NT)]

        extra = {i: [] for i in range(NC + 2)}
        def spread(tasks, rng):
            for i, part in zip(range(*rng), split(tasks, rng[1] - rng[0])):
                extra[i].extend(part)
        spread([functools.partial(router_tile, t) for t in range(X1 // 16)], (r_rng[0], f_at))
        spread([functools.partial(router_tile, t) for t in range(X1 // 16, S // 16)] + [router_fin], (f_at, r_rng[1]))
        spread([functools.partial(gate_up, f0) for f0 in range(0, F, FC)], gu_rng)

        qs_, os_, gs_ = {}, {}, {}

        def patch(lo, hi):
            if 'upd' not in st:
                y = jnp.sum(st['acc'], axis=0, keepdims=True) * sigmoid(st['mm'])
                g = sigmoid(jnp.sum(st['xrow'] * gw, axis=-1, keepdims=True))
                st['upd'] = (1.0 - g) * y
            t0 = pl.multiple_of(jnp.clip(st['t0'], lo, hi - 16), 16)
            sel = (t0 + lax.broadcasted_iota(jnp.int32, (16, 1), 0)) == st['idx']
            ot = out_v[pl.ds(t0, 16), :].astype(F32)
            out_v[pl.ds(t0, 16), :] = jnp.where(sel, ot + st['upd'], ot).astype(BF16)

        def tied(lhs, z):
            if z is None:
                return lhs
            u = pltpu.bitcast(lhs, U32)
            top = jnp.concatenate([u[:8, :128] | z, u[:8, 128:]], axis=1)
            return pltpu.bitcast(jnp.concatenate([top, u[8:]], axis=0), BF16)

        def proj(i, p, n0, z):
            r0 = i * CM
            n1 = min(n0 + NP, D)
            y = lax.dot_general(tied(x_v[r0:r0 + CM, :], z), pltpu.bitcast(wt_s[(p * D + n0) // 2:(p * D + n1) // 2, :], BF16),
                                NT_DIMS, preferred_element_type=F32)
            for jj in range((n1 - n0) // 128):
                j = n0 // 128 + jj
                yj = y[:, jj * 128:(jj + 1) * 128]
                if p == 0:
                    qs_[i, j] = yj
                    continue
                dst = (k_s if p == 1 else v_s)
                dst[i][j, HALO:HALO + CM, :] = yj
                if i + 1 < NC:
                    dst[i + 1][j, 0:HALO, :] = yj[CM - HALO:, :]
            return []

        def attn(i, b):
            r0 = i * CM
            ks, vs = k_s[i], v_s[i]
            qs = [qs_[i, j][b:b + RC, :] for j in range(NT)]
            ls = []
            for w in range(W):
                o = HALO + b - DIL * w
                acc = qs[0] * ks[0, o:o + RC, :]
                for j in range(1, NT):
                    acc = acc + qs[j] * ks[j, o:o + RC, :]
                acc = acc + pltpu.roll(acc, 64, 1)
                acc = acc + pltpu.roll(acc, 32, 1)
                if r0 + b < DIL * w:
                    pos = r0 + b + lax.broadcasted_iota(jnp.int32, (RC, 128), 0)
                    acc = jnp.where(pos >= DIL * w, acc, -1e9 * DH ** 0.5)
                ls.append(acc)
            mx = functools.reduce(jnp.maximum, ls)
            ps = [jnp.exp2((l - mx) * c) for l in ls]
            den = functools.reduce(jnp.add, ps)
            inv = pl.reciprocal(den, approx=True)
            inv = inv * (2.0 - den * inv)
            row = []
            for j in range(NT):
                acc = None
                for w in range(W):
                    o = HALO + b - DIL * w
                    t = ps[w] * vs[j, o:o + RC, :]
                    acc = t if acc is None else acc + t
                row.append(pltpu.bitcast((acc * inv).astype(BF16), U32))
            os_.setdefault(i, []).append(jnp.concatenate(row, axis=1))
            return row

        def gate(i):
            gs_[i] = sigmoid(jnp.sum(x_v[i * CM:(i + 1) * CM, :].astype(F32) * gw, axis=-1, keepdims=True))
            return []

        def outp(i, n0, z):
            r0 = i * CM
            n1 = min(n0 + NP, D)
            if n0 == 0:
                os_[i] = pltpu.bitcast(jnp.concatenate(os_[i], axis=0), BF16)
            a = jnp.dot(tied(os_[i], z), pltpu.bitcast(wop_s[:, n0:n1], BF16), preferred_element_type=F32)
            xf = x_v[r0:r0 + CM, n0:n1].astype(F32)
            g = gs_[i]
            res = (g * a + (1.0 - g) * xf).astype(BF16)
            out_v[r0:r0 + CM, n0:n1] = res
            ru = pltpu.bitcast(res, U32)
            if n1 == D and r0 + CM in ocuts[1:]:
                n = ocuts.index(r0 + CM) - 1
                if n >= NO - 2:
                    patch(ocuts[n] if n == NO - 1 else 0, ocuts[n + 1])
                cp_o[n].start()
                if n == NO - 2:
                    for cp in cp_o[:n]:
                        cp.wait()
                    tp = pl.multiple_of(jnp.where(st['idx'] < ocuts[n], st['t0'], 0), 16)
                    st['cp_p'] = pltpu.make_async_copy(out_v.at[pl.ds(tp, 16)], out_hbm.at[pl.ds(tp, 16)], sem_p.at[0])
                    st['cp_p'].start()
            return [ru[u * 8:(u + 1) * 8, jj * 128:(jj + 1) * 128] for u in range(CM // 16) for jj in range((n1 - n0) // 128)]

        due = {}
        clock = [0]

        def promise(toks, lag):
            due.setdefault(clock[0] + lag, []).extend(toks)

        def mxu(fn):
            toks = due.pop(clock[0], [])
            z = (functools.reduce(jnp.bitwise_or, toks) >> 31) >> 1 if toks and tie else None
            promise(fn(z), LM)
            clock[0] += 1

        wait_w(0)
        prep_w(0)
        with scope('wait_x0'):
            cp_x0.wait()
        for n in range(3):
            for i in range(P0):
                if i == P0 - 1:
                    if n < 2:
                        wait_w(n + 1)
                        prep_w(n + 1)
                    else:
                        with scope('wait_wo'):
                            cp_wo.wait()
                            cp_x1.wait()
                        cp_x2.start(priority=prio)
                        for cp in cp_f:
                            cp.start(priority=prio)
                        prep_wo()
                for n0 in range(0, D, NP):
                    mxu(functools.partial(proj, i, ORDER[n], n0))

        na = 0
        no = 0
        for i in range(P0, NC + 2):
            mm = []
            if i < NC:
                mm += [functools.partial(proj, i, p, n0) for p in ORDER for n0 in range(0, D, NP)]
            va = []
            while no < na and (no <= i - (2 if i < OL else 3) or i >= NC) and (i != NC or no < NC - 1):
                mm += [functools.partial(outp, no, n0) for n0 in range(0, D, NP)]
                va.append(functools.partial(gate, no))
                no += 1
            todo = []
            while na < min(i, NC) and len(todo) < (2 if (i - P0) % 2 == 1 or CU else 1):
                todo.append(na)
                na += 1
            at = split([functools.partial(attn, ci, b) for ci in todo for b in range(0, CM, RC)], len(mm))
            ex = split(extra.get(i, []), len(mm))
            ex[0] = va + ex[0]
            if i == f_at:
                with scope('wait_f'):
                    cp_x2.wait()
                    for cp in cp_f:
                        cp.wait()
            for n in range(len(mm)):
                for e in at[n]:
                    toks = e()
                    if i >= TF:
                        promise(toks, LA)
                for e in ex[n]:
                    promise(e(), LE)
                mxu(mm[n])

        with scope('wait_out'):
            cp_o[NO - 2].wait()
            st['cp_p'].wait()
            cp_o[NO - 1].wait()

    return kernel


def build(CM=128, RC=16, FC=64, NP=128, P0=3, x_at=1, f_at=8, r_rng=(4, 10), gu_rng=(10, 16), dn_rng=None,
          ocuts=(768, 1536, 1920), tie=True, prio=1, scopes=False, LA=4, LM=3, OL=15, CU=True, TF=14, LE=4, flags=None):
    def fn(A_x, A_wqkv, A_wo, B_x, B_w_r, B_w_gate, B_w_up, B_w_down, gate_w):
        x = A_x.reshape(S, D)
        any_spec = pl.BlockSpec(memory_space=pltpu.MemorySpace.HBM)
        vm = pl.BlockSpec(memory_space=pltpu.VMEM)
        out = pl.pallas_call(
            make_kernel(CM, RC, FC, NP, P0, x_at, f_at, r_rng, gu_rng, dn_rng, ocuts, tie, prio, scopes, LA, LM, OL, CU, TF, LE),
            out_shape=jax.ShapeDtypeStruct((S, D), BF16),
            in_specs=[any_spec, any_spec, any_spec, vm, any_spec, any_spec, any_spec, vm],
            out_specs=any_spec,
            scratch_shapes=[
                pltpu.VMEM((S, D), BF16), pltpu.VMEM((3, D, D), BF16), pltpu.VMEM((D, D), BF16),
                pltpu.VMEM((F, D), BF16), pltpu.VMEM((F, D), BF16), pltpu.VMEM((F, D), BF16),
                pltpu.VMEM((3, NT, D, 128), F32), pltpu.VMEM((3 * D // 2, D), U32), pltpu.VMEM((D // 2, D), U32),
                pltpu.VMEM((S, D), BF16),
                pltpu.SemaphoreType.DMA((4,)), pltpu.SemaphoreType.DMA((3,)), pltpu.SemaphoreType.DMA((3,)),
                pltpu.SemaphoreType.DMA((len(ocuts) + 1,)), pltpu.SemaphoreType.DMA((1,)),
            ] + [pltpu.VMEM((NT, CM + HALO, 128), F32)] * (2 * (S // CM)),
            compiler_params=pltpu.CompilerParams(vmem_limit_bytes=100 * 1024 * 1024, flags=flags),
        )(x, A_wqkv, A_wo, B_w_r, B_w_gate.T, B_w_up.T, B_w_down, gate_w)
        return out.reshape(1, S, D)
    return fn


_fn = build()


@jax.jit
def pallas_gated_mix__sliding_local_dilated__moe_arch_mod__prompt_kernel(
    A_x, A_wqkv, A_wo, B_x, B_w_r, B_w_gate, B_w_up, B_w_down, gate_w):
    return _fn(A_x, A_wqkv, A_wo, B_x, B_w_r, B_w_gate, B_w_up, B_w_down, gate_w)
```

```python
import functools
import math

import jax
import jax.numpy as jnp
from jax import lax
import jax.experimental.pallas as pl
import jax.experimental.pallas.tpu as pltpu

S, D, H, DH, W, DIL, F = 2048, 640, 32, 20, 8, 2, 1728
NT = D // 128
HALO = 16
CM = 128
NC = S // CM
RC = 16
FC = 64
P0 = 3
F_AT = 8
R_STEPS = (3, 11)
F_STEPS = (11, 16)
HOLD_AT = 15
PIN_AT = 14
OCUTS = (0, 768, 1664, 1920, S)
LAG_ATTN, LAG_MIX, LAG_EXTRA = 4, 3, 8
ORDER = (1, 2, 0)
F32, BF16, U32 = jnp.float32, jnp.bfloat16, jnp.uint32
NT_DIMS = (((1,), (1,)), ((), ()))


def _sigmoid(t):
    return 0.5 * jnp.tanh(0.5 * t) + 0.5


def _split(seq, n):
    seq = list(seq)
    return [seq[len(seq) * i // n:len(seq) * (i + 1) // n] for i in range(n)]


def _kernel(x_hbm, wqkv_hbm, wo_hbm, wr_hbm, wg_hbm, wu_hbm, wd_hbm, gw_hbm, out_hbm,
            wr_v, gw_v, x_v, wqkv_v, wo_v, wg_v, wu_v, wd_v, t_s, wt_s, wop_s, out_v,
            sem_w, sem_x, sem_f, sem_o, sem_p, *kv):
    k_s, v_s = kv[:NC], kv[NC:]
    copy = pltpu.make_async_copy
    no_seg = len(OCUTS) - 1
    xcuts = (0, P0 * CM, F_AT * CM, S)
    cp_w = [copy(wqkv_hbm.at[:, p * D:(p + 1) * D], wqkv_v.at[p], sem_w.at[p]) for p in range(3)]
    cp_wo = copy(wo_hbm, wo_v, sem_w.at[3])
    cp_x = [copy(x_hbm.at[pl.ds(a, b - a)], x_v.at[pl.ds(a, b - a)], sem_x.at[i])
            for i, (a, b) in enumerate(zip(xcuts[:-1], xcuts[1:]))]
    cp_f = [copy(a, b, sem_f.at[i])
            for i, (a, b) in enumerate(((wg_hbm, wg_v), (wu_hbm, wu_v), (wd_hbm, wd_v)))]
    cp_o = [copy(out_v.at[pl.ds(a, b - a)], out_hbm.at[pl.ds(a, b - a)], sem_o.at[i])
            for i, (a, b) in enumerate(zip(OCUTS[:-1], OCUTS[1:]))]
    cp_v = [copy(wr_hbm, wr_v, sem_w.at[4]), copy(gw_hbm, gw_v, sem_w.at[5])]

    cp_w[ORDER[0]].start()
    cp_x[0].start()
    cp_v[0].start()
    cp_v[1].start()
    cp_w[ORDER[1]].start(priority=1)

    for j in range(NT):
        k_s[0][j, 0:HALO, :] = jnp.zeros((HALO, 128), F32)
        v_s[0][j, 0:HALO, :] = jnp.zeros((HALO, 128), F32)

    def permute_rows(slot, dst, base):
        for j in range(NT):
            for d in range(DH):
                rows = t_s[slot, j, pl.ds(d, H, stride=DH), :].astype(BF16)
                dst[pl.ds((base + d * H) // 2, H // 2), j * 128:(j + 1) * 128] = pltpu.bitcast(rows, U32)

    def prep_w(n):
        p = ORDER[n]
        for j in range(NT):
            t_s[n, j] = wqkv_v[p, j * 128:(j + 1) * 128, :].astype(F32).T
        permute_rows(n, wt_s, p * D)

    def prep_wo():
        for j in range(NT):
            t_s[0, j] = wo_v[:, j * 128:(j + 1) * 128].astype(F32)
        permute_rows(0, wop_s, 0)

    st = dict(m=jnp.full((8, 1), -jnp.inf, F32), bi=jnp.zeros((8, 1), jnp.int32),
              acc=jnp.zeros((8, D), F32))
    sub = lax.broadcasted_iota(jnp.int32, (8, 1), 0)

    def router_tile(t):
        xs = x_v[t * 16:(t + 1) * 16, :].astype(F32)
        r = jnp.sum(xs * st['wr'], axis=-1, keepdims=True).astype(BF16).astype(F32)
        for hh in range(2):
            rr = r[hh * 8:(hh + 1) * 8]
            better = rr > st['m']
            st['m'] = jnp.where(better, rr, st['m'])
            st['bi'] = jnp.where(better, sub + (t * 16 + hh * 8), st['bi'])
        return [pltpu.bitcast(jnp.broadcast_to(st['bi'], (8, 128)), U32)]

    def router_fin():
        top = jnp.max(st['m'], axis=0, keepdims=True)
        first = jnp.min(jnp.where(st['m'] == top, st['bi'], S), axis=0, keepdims=True)
        idx = jnp.clip(first[0, 0], 0, S - 1)
        t0 = pl.multiple_of((idx // 16) * 16, 16)
        xt = x_v[pl.ds(t0, 16), :].astype(F32)
        sel = (t0 + lax.broadcasted_iota(jnp.int32, (16, 1), 0)) == idx
        xrow = jnp.sum(jnp.where(sel, xt, 0.0), axis=0, keepdims=True)
        st.update(top=top, idx=idx, t0=t0, xrow=xrow)
        return [pltpu.bitcast(jnp.broadcast_to(xrow[:, :128], (8, 128)), U32)]

    def ffn(f0):
        gg = jnp.sum(wg_v[f0:f0 + FC, :].astype(F32) * st['xrow'], axis=-1, keepdims=True)
        uu = jnp.sum(wu_v[f0:f0 + FC, :].astype(F32) * st['xrow'], axis=-1, keepdims=True)
        hh = gg * _sigmoid(gg) * uu
        t = wd_v[f0:f0 + FC, :].astype(F32) * hh
        for u in range(FC // 8):
            st['acc'] = st['acc'] + t[u * 8:(u + 1) * 8]
        return [pltpu.bitcast(st['acc'][:, j * 128:(j + 1) * 128], U32) for j in range(NT)]

    def patch(lo, hi):
        if 'upd' not in st:
            y = jnp.sum(st['acc'], axis=0, keepdims=True) * _sigmoid(st['top'])
            g = _sigmoid(jnp.sum(st['xrow'] * st['gw'], axis=-1, keepdims=True))
            st['upd'] = (1.0 - g) * y
        t0 = pl.multiple_of(jnp.clip(st['t0'], lo, hi - 16), 16)
        sel = (t0 + lax.broadcasted_iota(jnp.int32, (16, 1), 0)) == st['idx']
        ot = out_v[pl.ds(t0, 16), :].astype(F32)
        out_v[pl.ds(t0, 16), :] = jnp.where(sel, ot + st['upd'], ot).astype(BF16)

    extra = {i: [] for i in range(NC + 2)}

    def spread(tasks, lo, hi):
        for i, part in zip(range(lo, hi), _split(tasks, hi - lo)):
            extra[i].extend(part)

    spread([functools.partial(router_tile, t) for t in range(xcuts[2] // 16)], R_STEPS[0], F_AT)
    spread([functools.partial(router_tile, t) for t in range(xcuts[2] // 16, S // 16)] + [router_fin],
           F_AT, R_STEPS[1])
    spread([functools.partial(ffn, f0) for f0 in range(0, F, FC)], *F_STEPS)

    q_of, o_of, g_of = {}, {}, {}
    exp_scale = (DH ** -0.5) * math.log2(math.e)

    def after(lhs, z):
        if z is None:
            return lhs
        u = pltpu.bitcast(lhs, U32)
        top = jnp.concatenate([u[:8, :128] | z, u[:8, 128:]], axis=1)
        return pltpu.bitcast(jnp.concatenate([top, u[8:]], axis=0), BF16)

    def proj(i, p, j, z):
        n0 = (p * D + j * 128) // 2
        y = lax.dot_general(after(x_v[i * CM:(i + 1) * CM, :], z),
                            pltpu.bitcast(wt_s[n0:n0 + 64, :], BF16), NT_DIMS,
                            preferred_element_type=F32)
        if p == 0:
            q_of[i, j] = y
        else:
            dst = k_s if p == 1 else v_s
            dst[i][j, HALO:HALO + CM, :] = y
            if i + 1 < NC:
                dst[i + 1][j, 0:HALO, :] = y[CM - HALO:, :]
        return []

    def attn(i, b):
        r0 = i * CM + b
        qs = [q_of[i, j][b:b + RC, :] for j in range(NT)]
        logits = []
        for w in range(W):
            o = HALO + b - DIL * w
            acc = qs[0] * k_s[i][0, o:o + RC, :]
            for j in range(1, NT):
                acc = acc + qs[j] * k_s[i][j, o:o + RC, :]
            acc = acc + pltpu.roll(acc, 64, 1)
            acc = acc + pltpu.roll(acc, 32, 1)
            if r0 < DIL * w:
                pos = r0 + lax.broadcasted_iota(jnp.int32, (RC, 128), 0)
                acc = jnp.where(pos >= DIL * w, acc, -1e9 * DH ** 0.5)
            logits.append(acc)
        mx = functools.reduce(jnp.maximum, logits)
        ps = [jnp.exp2((l - mx) * exp_scale) for l in logits]
        den = functools.reduce(jnp.add, ps)
        inv = pl.reciprocal(den, approx=True)
        inv = inv * (2.0 - den * inv)
        row = []
        for j in range(NT):
            acc = None
            for w in range(W):
                o = HALO + b - DIL * w
                t = ps[w] * v_s[i][j, o:o + RC, :]
                acc = t if acc is None else acc + t
            row.append(pltpu.bitcast((acc * inv).astype(BF16), U32))
        o_of.setdefault(i, []).append(jnp.concatenate(row, axis=1))
        return row

    def gate(i):
        xs = x_v[i * CM:(i + 1) * CM, :].astype(F32)
        g_of[i] = _sigmoid(jnp.sum(xs * st['gw'], axis=-1, keepdims=True))

    def outp(i, j, z):
        r0, n0 = i * CM, j * 128
        if j == 0:
            o_of[i] = pltpu.bitcast(jnp.concatenate(o_of[i], axis=0), BF16)
        a = jnp.dot(after(o_of[i], z), pltpu.bitcast(wop_s[:, n0:n0 + 128], BF16),
                    preferred_element_type=F32)
        xf = x_v[r0:r0 + CM, n0:n0 + 128].astype(F32)
        g = g_of[i]
        res = (g * a + (1.0 - g) * xf).astype(BF16)
        out_v[r0:r0 + CM, n0:n0 + 128] = res
        ru = pltpu.bitcast(res, U32)
        if j == NT - 1 and r0 + CM in OCUTS[1:]:
            n = OCUTS.index(r0 + CM) - 1
            if n == no_seg - 2:
                for cp in cp_o[:n]:
                    cp.wait()
            if n >= no_seg - 2:
                patch(OCUTS[n] if n == no_seg - 1 else 0, OCUTS[n + 1])
            cp_o[n].start()
            if n == no_seg - 2:
                tp = pl.multiple_of(jnp.where(st['idx'] < OCUTS[n], st['t0'], 0), 16)
                st['cp_p'] = copy(out_v.at[pl.ds(tp, 16)], out_hbm.at[pl.ds(tp, 16)], sem_p.at[0])
                st['cp_p'].start()
        return [ru[u * 8:(u + 1) * 8, :] for u in range(CM // 16)]

    due = {}
    clock = [0]

    def promise(values, lag):
        due.setdefault(clock[0] + lag, []).extend(values)

    def mxu(piece):
        values = due.pop(clock[0], [])
        z = (functools.reduce(jnp.bitwise_or, values) >> 31) >> 1 if values else None
        promise(piece(z), LAG_MIX)
        clock[0] += 1

    cp_w[ORDER[0]].wait()
    cp_w[ORDER[2]].start(priority=1)
    prep_w(0)
    cp_x[0].wait()
    for n in range(3):
        for i in range(P0):
            if i == P0 - 1:
                if n < 2:
                    cp_w[ORDER[n + 1]].wait()
                    if n == 0:
                        cp_wo.start(priority=1)
                        cp_x[1].start(priority=1)
                    else:
                        cp_v[0].wait()
                        cp_v[1].wait()
                        st['wr'] = wr_v[...].astype(F32).reshape(1, D)
                        st['gw'] = gw_v[...].astype(F32).reshape(1, D)
                        gate(0)
                    prep_w(n + 1)
                else:
                    cp_wo.wait()
                    cp_x[1].wait()
                    cp_x[2].start(priority=1)
                    for cp in cp_f:
                        cp.start(priority=1)
                    prep_wo()
            early = _split(range(0, CM, RC), NT) if (n, i) == (2, 1) else [[]] * NT
            for j in range(NT):
                for b in early[j]:
                    promise(attn(0, b), LAG_ATTN)
                mxu(functools.partial(proj, i, ORDER[n], j))

    n_attn, n_out = 1, 0
    for i in range(P0, NC + 2):
        pieces = []
        if i < NC:
            pieces = [functools.partial(proj, i, p, j) for p in ORDER for j in range(NT)]
        outs = []
        while (n_out < NC and len(outs) < 2 and (i != NC or n_out < NC - 1)
               and (i >= NC or n_out <= i - (2 if i < HOLD_AT else 3))):
            outs.append(n_out)
            n_out += 1
        late, pinned = [], []
        while n_attn < min(i, NC) and (n_attn < n_out or i >= PIN_AT):
            (late if n_attn < n_out else pinned).append(n_attn)
            n_attn += 1
        op = [[functools.partial(outp, ci, j) for j in range(NT)] for ci in outs]
        if len(op) == 2:
            pieces = pieces[:NT] + op[0] + pieces[NT:] + op[1]
        else:
            pieces = pieces + sum(op, [])
        groups = _split([(ci, b) for ci in pinned for b in range(0, CM, RC)], len(pieces))
        others = _split(extra[i], len(pieces))
        if i == F_AT:
            cp_x[2].wait()
            for cp in cp_f:
                cp.wait()
        for ci in late:
            for b in range(0, CM, RC):
                attn(ci, b)
        for ci in outs:
            if ci not in g_of:
                gate(ci)
        for n, piece in enumerate(pieces):
            for ci, b in groups[n]:
                promise(attn(ci, b), LAG_ATTN)
            for task in others[n]:
                promise(task(), LAG_EXTRA)
            mxu(piece)

    cp_o[no_seg - 2].wait()
    st['cp_p'].wait()
    cp_o[no_seg - 1].wait()


@jax.jit
def pallas_gated_mix__sliding_local_dilated__moe_arch_mod__prompt_kernel(
    A_x: jax.Array,
    A_wqkv: jax.Array,
    A_wo: jax.Array,
    B_x: jax.Array,
    B_w_r: jax.Array,
    B_w_gate: jax.Array,
    B_w_up: jax.Array,
    B_w_down: jax.Array,
    gate_w: jax.Array,
):
    del B_x
    hbm = pl.BlockSpec(memory_space=pltpu.MemorySpace.HBM)
    dma = pltpu.SemaphoreType.DMA
    out = pl.pallas_call(
        _kernel,
        out_shape=jax.ShapeDtypeStruct((S, D), BF16),
        in_specs=[hbm] * 8,
        out_specs=hbm,
        scratch_shapes=[
            pltpu.VMEM((D,), BF16), pltpu.VMEM((D,), BF16),
            pltpu.VMEM((S, D), BF16), pltpu.VMEM((3, D, D), BF16), pltpu.VMEM((D, D), BF16),
            pltpu.VMEM((F, D), BF16), pltpu.VMEM((F, D), BF16), pltpu.VMEM((F, D), BF16),
            pltpu.VMEM((3, NT, D, 128), F32),
            pltpu.VMEM((3 * D // 2, D), U32), pltpu.VMEM((D // 2, D), U32),
            pltpu.VMEM((S, D), BF16),
            dma((6,)), dma((3,)), dma((3,)), dma((len(OCUTS) - 1,)), dma((1,)),
        ] + [pltpu.VMEM((NT, CM + HALO, 128), F32)] * (2 * NC),
        compiler_params=pltpu.CompilerParams(vmem_limit_bytes=100 * 1024 * 1024),
    )(A_x.reshape(S, D), A_wqkv, A_wo, B_w_r, B_w_gate.T, B_w_up.T, B_w_down, gate_w)
    return out.reshape(1, S, D)
```

```python
import functools
import math

import jax
import jax.numpy as jnp
from jax import lax
import jax.experimental.pallas as pl
import jax.experimental.pallas.tpu as pltpu

S, D, H, DH, W, DIL, F = 2048, 640, 32, 20, 8, 2, 1728
NT = D // 128
HALO = 16
CM = 128
NC = S // CM
RC = 16
FC = 64
P0 = 3
F_AT = 8
R_STEPS = (3, 11)
F_STEPS = (11, 16)
HOLD_AT = 15
PIN_AT = 14
OCUTS = (0, 768, 1664, 1920, S)
LAG_ATTN, LAG_MIX, LAG_EXTRA = 4, 4, 8
PIN_GROUPS, PIN_LAG = 4, 7
ORDER = (1, 2, 0)
F32, BF16, U32 = jnp.float32, jnp.bfloat16, jnp.uint32
NT_DIMS = (((1,), (1,)), ((), ()))


def _sigmoid(t):
    return 0.5 * jnp.tanh(0.5 * t) + 0.5


def _split(seq, n):
    seq = list(seq)
    return [seq[len(seq) * i // n:len(seq) * (i + 1) // n] for i in range(n)]


def _kernel(x_hbm, wqkv_hbm, wo_hbm, wr_hbm, wg_hbm, wu_hbm, wd_hbm, gw_hbm, out_hbm,
            wr_v, gw_v, x_v, wqkv_v, wo_v, wg_v, wu_v, wd_v, t_s, wt_s, wop_s, out_v,
            sem_w, sem_x, sem_f, sem_o, sem_p, *kv):
    k_s, v_s = kv[:NC], kv[NC:]
    copy = pltpu.make_async_copy
    no_seg = len(OCUTS) - 1
    xcuts = (0, P0 * CM, F_AT * CM, S)
    cp_w = [copy(wqkv_hbm.at[:, p * D:(p + 1) * D], wqkv_v.at[p], sem_w.at[p]) for p in range(3)]
    cp_wo = copy(wo_hbm, wo_v, sem_w.at[3])
    cp_x = [copy(x_hbm.at[pl.ds(a, b - a)], x_v.at[pl.ds(a, b - a)], sem_x.at[i])
            for i, (a, b) in enumerate(zip(xcuts[:-1], xcuts[1:]))]
    cp_f = [copy(a, b, sem_f.at[i])
            for i, (a, b) in enumerate(((wg_hbm, wg_v), (wu_hbm, wu_v), (wd_hbm, wd_v)))]
    cp_o = [copy(out_v.at[pl.ds(a, b - a)], out_hbm.at[pl.ds(a, b - a)], sem_o.at[i])
            for i, (a, b) in enumerate(zip(OCUTS[:-1], OCUTS[1:]))]
    cp_v = [copy(wr_hbm, wr_v, sem_w.at[4]), copy(gw_hbm, gw_v, sem_w.at[5])]

    cp_w[ORDER[0]].start()
    cp_x[0].start()
    cp_v[0].start()
    cp_v[1].start()
    cp_w[ORDER[1]].start(priority=1)

    for j in range(NT):
        k_s[0][j, 0:HALO, :] = jnp.zeros((HALO, 128), F32)
        v_s[0][j, 0:HALO, :] = jnp.zeros((HALO, 128), F32)

    def permute_rows(slot, dst, base):
        for j in range(NT):
            for d in range(DH):
                rows = t_s[slot, j, pl.ds(d, H, stride=DH), :].astype(BF16)
                dst[pl.ds((base + d * H) // 2, H // 2), j * 128:(j + 1) * 128] = pltpu.bitcast(rows, U32)

    def prep_w(n):
        p = ORDER[n]
        for j in range(NT):
            t_s[n, j] = wqkv_v[p, j * 128:(j + 1) * 128, :].astype(F32).T
        permute_rows(n, wt_s, p * D)

    def prep_wo():
        for j in range(NT):
            t_s[0, j] = wo_v[:, j * 128:(j + 1) * 128].astype(F32)
        permute_rows(0, wop_s, 0)

    st = dict(m=jnp.full((8, 1), -jnp.inf, F32), bi=jnp.zeros((8, 1), jnp.int32),
              acc=jnp.zeros((8, D), F32))
    sub = lax.broadcasted_iota(jnp.int32, (8, 1), 0)

    def router_tile(t):
        xs = x_v[t * 16:(t + 1) * 16, :].astype(F32)
        r = jnp.sum(xs * st['wr'], axis=-1, keepdims=True).astype(BF16).astype(F32)
        for hh in range(2):
            rr = r[hh * 8:(hh + 1) * 8]
            better = rr > st['m']
            st['m'] = jnp.where(better, rr, st['m'])
            st['bi'] = jnp.where(better, sub + (t * 16 + hh * 8), st['bi'])
        return [pltpu.bitcast(jnp.broadcast_to(st['bi'], (8, 128)), U32)]

    def router_fin():
        top = jnp.max(st['m'], axis=0, keepdims=True)
        first = jnp.min(jnp.where(st['m'] == top, st['bi'], S), axis=0, keepdims=True)
        idx = jnp.clip(first[0, 0], 0, S - 1)
        t0 = pl.multiple_of((idx // 16) * 16, 16)
        xt = x_v[pl.ds(t0, 16), :].astype(F32)
        sel = (t0 + lax.broadcasted_iota(jnp.int32, (16, 1), 0)) == idx
        xrow = jnp.sum(jnp.where(sel, xt, 0.0), axis=0, keepdims=True)
        st.update(top=top, idx=idx, t0=t0, xrow=xrow)
        return [pltpu.bitcast(jnp.broadcast_to(xrow[:, :128], (8, 128)), U32)]

    def ffn(f0):
        gg = jnp.sum(wg_v[f0:f0 + FC, :].astype(F32) * st['xrow'], axis=-1, keepdims=True)
        uu = jnp.sum(wu_v[f0:f0 + FC, :].astype(F32) * st['xrow'], axis=-1, keepdims=True)
        hh = gg * _sigmoid(gg) * uu
        t = wd_v[f0:f0 + FC, :].astype(F32) * hh
        for u in range(FC // 8):
            st['acc'] = st['acc'] + t[u * 8:(u + 1) * 8]
        return [pltpu.bitcast(st['acc'][:, j * 128:(j + 1) * 128], U32) for j in range(NT)]

    def patch(lo, hi):
        if 'upd' not in st:
            y = jnp.sum(st['acc'], axis=0, keepdims=True) * _sigmoid(st['top'])
            g = _sigmoid(jnp.sum(st['xrow'] * st['gw'], axis=-1, keepdims=True))
            st['upd'] = (1.0 - g) * y
        t0 = pl.multiple_of(jnp.clip(st['t0'], lo, hi - 16), 16)
        sel = (t0 + lax.broadcasted_iota(jnp.int32, (16, 1), 0)) == st['idx']
        ot = out_v[pl.ds(t0, 16), :].astype(F32)
        out_v[pl.ds(t0, 16), :] = jnp.where(sel, ot + st['upd'], ot).astype(BF16)

    extra = {i: [] for i in range(NC + 2)}

    def spread(tasks, lo, hi):
        for i, part in zip(range(lo, hi), _split(tasks, hi - lo)):
            extra[i].extend(part)

    spread([functools.partial(router_tile, t) for t in range(xcuts[2] // 16)], R_STEPS[0], F_AT)
    spread([functools.partial(router_tile, t) for t in range(xcuts[2] // 16, S // 16)] + [router_fin],
           F_AT, R_STEPS[1])
    spread([functools.partial(ffn, f0) for f0 in range(0, F, FC)], *F_STEPS)

    q_of, o_of, g_of = {}, {}, {}
    exp_scale = (DH ** -0.5) * math.log2(math.e)

    def after(lhs, z):
        if z is None:
            return lhs
        u = pltpu.bitcast(lhs, U32)
        top = jnp.concatenate([u[:8, :128] | z, u[:8, 128:]], axis=1)
        return pltpu.bitcast(jnp.concatenate([top, u[8:]], axis=0), BF16)

    def proj(i, p, j, z):
        n0 = (p * D + j * 128) // 2
        y = lax.dot_general(after(x_v[i * CM:(i + 1) * CM, :], z),
                            pltpu.bitcast(wt_s[n0:n0 + 64, :], BF16), NT_DIMS,
                            preferred_element_type=F32)
        if p == 0:
            q_of[i, j] = y
        else:
            dst = k_s if p == 1 else v_s
            dst[i][j, HALO:HALO + CM, :] = y
            if i + 1 < NC:
                dst[i + 1][j, 0:HALO, :] = y[CM - HALO:, :]
        return []

    def attn(i, b):
        r0 = i * CM + b
        qs = [q_of[i, j][b:b + RC, :] for j in range(NT)]
        logits = []
        for w in range(W):
            o = HALO + b - DIL * w
            acc = qs[0] * k_s[i][0, o:o + RC, :]
            for j in range(1, NT):
                acc = acc + qs[j] * k_s[i][j, o:o + RC, :]
            acc = acc + pltpu.roll(acc, 64, 1)
            acc = acc + pltpu.roll(acc, 32, 1)
            if r0 < DIL * w:
                pos = r0 + lax.broadcasted_iota(jnp.int32, (RC, 128), 0)
                acc = jnp.where(pos >= DIL * w, acc, -1e9 * DH ** 0.5)
            logits.append(acc)
        mx = functools.reduce(jnp.maximum, logits)
        ps = [jnp.exp2((l - mx) * exp_scale) for l in logits]
        den = functools.reduce(jnp.add, ps)
        inv = pl.reciprocal(den, approx=True)
        inv = inv * (2.0 - den * inv)
        row = []
        for j in range(NT):
            acc = None
            for w in range(W):
                o = HALO + b - DIL * w
                t = ps[w] * v_s[i][j, o:o + RC, :]
                acc = t if acc is None else acc + t
            row.append(pltpu.bitcast((acc * inv).astype(BF16), U32))
        o_of.setdefault(i, []).append(jnp.concatenate(row, axis=1))
        return row

    def gate(i):
        xs = x_v[i * CM:(i + 1) * CM, :].astype(F32)
        g_of[i] = _sigmoid(jnp.sum(xs * st['gw'], axis=-1, keepdims=True))

    def outp(i, j, z):
        r0, n0 = i * CM, j * 128
        if j == 0:
            o_of[i] = pltpu.bitcast(jnp.concatenate(o_of[i], axis=0), BF16)
        a = jnp.dot(after(o_of[i], z), pltpu.bitcast(wop_s[:, n0:n0 + 128], BF16),
                    preferred_element_type=F32)
        xf = x_v[r0:r0 + CM, n0:n0 + 128].astype(F32)
        g = g_of[i]
        res = (g * a + (1.0 - g) * xf).astype(BF16)
        out_v[r0:r0 + CM, n0:n0 + 128] = res
        ru = pltpu.bitcast(res, U32)
        if j == NT - 1 and r0 + CM in OCUTS[1:]:
            n = OCUTS.index(r0 + CM) - 1
            if n == no_seg - 2:
                for cp in cp_o[:n]:
                    cp.wait()
            if n >= no_seg - 2:
                patch(OCUTS[n] if n == no_seg - 1 else 0, OCUTS[n + 1])
            cp_o[n].start()
            if n == no_seg - 2:
                tp = pl.multiple_of(jnp.where(st['idx'] < OCUTS[n], st['t0'], 0), 16)
                st['cp_p'] = copy(out_v.at[pl.ds(tp, 16)], out_hbm.at[pl.ds(tp, 16)], sem_p.at[0])
                st['cp_p'].start()
        return [ru[u * 8:(u + 1) * 8, :] for u in range(CM // 16)]

    due = {}
    clock = [0]

    def promise(values, lag):
        due.setdefault(clock[0] + lag, []).extend(values)

    def mxu(piece):
        values = due.pop(clock[0], [])
        z = (functools.reduce(jnp.bitwise_or, values) >> 31) >> 1 if values else None
        promise(piece(z), LAG_MIX)
        clock[0] += 1

    cp_w[ORDER[0]].wait()
    cp_w[ORDER[2]].start(priority=1)
    prep_w(0)
    cp_x[0].wait()
    for n in range(3):
        for i in range(P0):
            if i == P0 - 1:
                if n < 2:
                    cp_w[ORDER[n + 1]].wait()
                    if n == 0:
                        cp_wo.start(priority=1)
                        cp_x[1].start(priority=1)
                    else:
                        cp_v[0].wait()
                        cp_v[1].wait()
                        st['wr'] = wr_v[...].astype(F32).reshape(1, D)
                        st['gw'] = gw_v[...].astype(F32).reshape(1, D)
                        gate(0)
                    prep_w(n + 1)
                else:
                    cp_wo.wait()
                    cp_x[1].wait()
                    cp_x[2].start(priority=1)
                    for cp in cp_f:
                        cp.start(priority=1)
                    prep_wo()
            early = _split(range(0, CM, RC), NT) if (n, i) == (2, 1) else [[]] * NT
            for j in range(NT):
                for b in early[j]:
                    promise(attn(0, b), LAG_ATTN)
                mxu(functools.partial(proj, i, ORDER[n], j))

    n_attn, n_out = 1, 0
    for i in range(P0, NC + 2):
        pieces = []
        if i < NC:
            pieces = [functools.partial(proj, i, p, j) for p in ORDER for j in range(NT)]
        outs = []
        while (n_out < NC and len(outs) < 2 and (i != NC or n_out < NC - 1)
               and (i >= NC or n_out <= i - (2 if i < HOLD_AT else 3))):
            outs.append(n_out)
            n_out += 1
        late, pinned = [], []
        while n_attn < min(i, NC) and (n_attn < n_out or i >= PIN_AT):
            (late if n_attn < n_out else pinned).append(n_attn)
            n_attn += 1
        op = [[functools.partial(outp, ci, j) for j in range(NT)] for ci in outs]
        if len(op) == 2:
            pieces = pieces[:2 * NT] + op[0] + pieces[2 * NT:] + op[1]
        else:
            pieces = pieces + sum(op, [])
        groups = _split([(ci, b) for ci in pinned for b in range(0, CM, RC)], len(pieces))
        others = _split(extra[i], len(pieces))
        if i == F_AT:
            cp_x[2].wait()
            for cp in cp_f:
                cp.wait()
        for ci in late:
            for n, b in enumerate(range(0, CM, RC)):
                values = attn(ci, b)
                if n < PIN_GROUPS and len(outs) == 1:
                    promise(values, PIN_LAG + n)
        for ci in outs:
            if ci not in g_of:
                gate(ci)
        for n, piece in enumerate(pieces):
            for ci, b in groups[n]:
                promise(attn(ci, b), LAG_ATTN)
            for task in others[n]:
                promise(task(), LAG_EXTRA)
            mxu(piece)

    cp_o[no_seg - 2].wait()
    st['cp_p'].wait()
    cp_o[no_seg - 1].wait()


@jax.jit
def pallas_gated_mix__sliding_local_dilated__moe_arch_mod__prompt_kernel(
    A_x: jax.Array,
    A_wqkv: jax.Array,
    A_wo: jax.Array,
    B_x: jax.Array,
    B_w_r: jax.Array,
    B_w_gate: jax.Array,
    B_w_up: jax.Array,
    B_w_down: jax.Array,
    gate_w: jax.Array,
):
    del B_x
    hbm = pl.BlockSpec(memory_space=pltpu.MemorySpace.HBM)
    dma = pltpu.SemaphoreType.DMA
    out = pl.pallas_call(
        _kernel,
        out_shape=jax.ShapeDtypeStruct((S, D), BF16),
        in_specs=[hbm] * 8,
        out_specs=hbm,
        scratch_shapes=[
            pltpu.VMEM((D,), BF16), pltpu.VMEM((D,), BF16),
            pltpu.VMEM((S, D), BF16), pltpu.VMEM((3, D, D), BF16), pltpu.VMEM((D, D), BF16),
            pltpu.VMEM((F, D), BF16), pltpu.VMEM((F, D), BF16), pltpu.VMEM((F, D), BF16),
            pltpu.VMEM((3, NT, D, 128), F32),
            pltpu.VMEM((3 * D // 2, D), U32), pltpu.VMEM((D // 2, D), U32),
            pltpu.VMEM((S, D), BF16),
            dma((6,)), dma((3,)), dma((3,)), dma((len(OCUTS) - 1,)), dma((1,)),
        ] + [pltpu.VMEM((NT, CM + HALO, 128), F32)] * (2 * NC),
        compiler_params=pltpu.CompilerParams(vmem_limit_bytes=100 * 1024 * 1024),
    )(A_x.reshape(S, D), A_wqkv, A_wo, B_w_r, B_w_gate.T, B_w_up.T, B_w_down, gate_w)
    return out.reshape(1, S, D)
```
